```python
import os as _os
_os.environ.setdefault("JAX_PLATFORMS", "cpu")
import jax
import jax.numpy as jnp

def _softmax(x, axis=-1):
    return jax.nn.softmax(x, axis=axis)
def _gelu(x):
    return jax.nn.gelu(x, approximate=True)
def _silu(x):
    return jax.nn.silu(x)
def _sigmoid(x):
    return jax.nn.sigmoid(x)
def _layernorm(x, axis=-1, eps=1e-5):
    m = jnp.mean(x, axis=axis, keepdims=True)
    v = jnp.var(x, axis=axis, keepdims=True)
    return (x - m) / jnp.sqrt(v + eps)
def _scatter_add(tgt, idx, src, axis=0):
    return tgt.at[idx].add(src)
def _segment_sum(src, seg, n):
    return jax.ops.segment_sum(src, seg, n)
class _Rng:
    def __init__(self, key):
        self._k = key
    def _next(self):
        self._k, sub = jax.random.split(self._k)
        return sub
    def normal(self, shape):
        return jax.random.normal(self._next(), shape, dtype=jnp.bfloat16)
    def randint(self, lo, hi, shape):
        return jax.random.randint(self._next(), shape, lo, hi, dtype=jnp.int32)
    def uniform(self, shape, lo=0.0, hi=1.0):
        return jax.random.uniform(self._next(), shape, jnp.bfloat16, lo, hi)
    def permutation(self, n):
        return jax.random.permutation(self._next(), n)


kernel_name = 'concat_heads__ssm_conv_h3__sliding_block__prompt'

def setup_inputs():
    _rng = _Rng(jax.random.key(int.from_bytes(__import__("os").urandom(4), "little")))
    _w = (lambda a: (lambda t: t.astype(jnp.bfloat16) if jnp.issubdtype(t.dtype, jnp.floating) else t)(jnp.asarray(a)))
    def _A_setup():
        B, S, D = 1, 2048, 512
        ks = 4
        return {
            "q": _w((lambda *s: _rng.normal(s) * 0.05)(B, S, D)),
            "k": _w((lambda *s: _rng.normal(s) * 0.2)(B, S, D)),
            "v": _w((lambda *s: _rng.normal(s) * 0.2)(B, S, D)),
            "shift_k": _w((lambda *s: _rng.normal(s) * 0.2)(D, ks) * 0.5),
            "ssm_k": _w((lambda *s: _rng.normal(s) * 0.2)(D, S) * (1.0 / S ** 0.5)),
            "ssm_D": _w((lambda *s: _rng.normal(s) * 0.2)(D)),
        }
    _A_in = _A_setup()

    def _B_setup():
        B, S, D = 1, 2048, 512
        return {
            "x": _w((lambda *s: _rng.normal(s) * 0.2)(B, S, D)),
            "wqkv": _w((lambda *s: _rng.normal(s) * 0.2)(D, 3 * D)),
            "wo": _w((lambda *s: _rng.normal(s) * 0.05)(D, D)),
        }
    _B_in = _B_setup()

    return {
        "A_q": _A_in["q"],
        "A_k": _A_in["k"],
        "A_v": _A_in["v"],
        "A_shift_k": _A_in["shift_k"],
        "A_ssm_k": _A_in["ssm_k"],
        "A_ssm_D": _A_in["ssm_D"],
        "B_x": _B_in["x"],
        "B_wqkv": _B_in["wqkv"],
        "B_wo": _B_in["wo"],
    }

def reference(A_q, A_k, A_v, A_shift_k, A_ssm_k, A_ssm_D, B_x, B_wqkv, B_wo):
    def _A_ref(q, k, v, shift_k, ssm_k, ssm_D):
        B, S, D = q.shape
        ks = shift_k.shape[-1]
        k_pad = jnp.pad(k, ((0, 0), (ks - 1, 0), (0, 0)))
        k_shift = jnp.zeros_like(k)
        for t in range(ks):
            k_shift = k_shift + k_pad[:, t:t + S, :] * shift_k[:, ks - 1 - t][None, None, :]
        kv = k_shift * v
        L = 2 * S
        kv_pad = jnp.pad(kv, ((0, 0), (0, S), (0, 0)))
        kf_pad = jnp.pad(ssm_k, ((0, 0), (0, S)))
        kv_f = (lambda x, axes=(-2,-1): jnp.fft.rfft2(x.astype(jnp.float32), axes=axes))(kv_pad[:, None, :, :], axes=(1, 2))
        kf_f = (lambda x, axes=(-2,-1): jnp.fft.rfft2(x.astype(jnp.float32), axes=axes))(kf_pad[:, None, :], axes=(1, 2))
        kf_f = (lambda x, *d: x.transpose(*d))(kf_f, 1, 2, 0)
        y_f = kv_f * kf_f[None, :, :, :]
        y = (lambda x, s, axes=(-2,-1): jnp.fft.irfft2(x, s=s, axes=axes).astype(jnp.bfloat16))(y_f, (1, L), axes=(1, 2))[:, 0, :S, :]
        y = y + kv * ssm_D[None, None, :]
        return q * y

    def _B_ref(x, wqkv, wo):
        B, S, D = x.shape
        H = 32; Dh = D // H; W = 256
        qkv = (lambda x, *d: x.transpose(*d))((x @ wqkv).reshape(B, S, 3, H, Dh), 2, 0, 3, 1, 4)
        q, k, v = qkv[0], qkv[1], qkv[2]
        scores = jnp.einsum("bhqd,bhkd->bhqk", q, k) * (Dh ** -0.5)
        idx = jnp.arange(S)
        mask = (idx[:, None] - idx[None, :] >= 0) & (idx[:, None] - idx[None, :] < W)
        scores = jnp.where(mask[None, None], scores, -1e9)
        p = _softmax(scores, axis=-1)
        o = jnp.einsum("bhqk,bhkd->bhqd", p, v)
        return (lambda x, *d: x.transpose(*d))(o, 0, 2, 1, 3).reshape(B, S, D) @ wo

    a = _A_ref(A_q, A_k, A_v, A_shift_k, A_ssm_k, A_ssm_D)
    b = _B_ref(B_x, B_wqkv, B_wo)
    return jnp.concatenate([a, b], axis=-1)
```

```python
import math
import numpy as np
import jax
import jax.numpy as jnp
from jax import lax
import jax.experimental.pallas as pl
import jax.experimental.pallas.tpu as pltpu

S = 2048
D = 512
H = 32
DH = 16
BQ = 128
RB = 256
NSTEP = S // RB
NB = S // 128
BIG = 1e30
QSCALE = (DH ** -0.5) * math.log2(math.e)
NCH = 1
CR = 64 // NCH
Q_OFF, U_OFF, G_OFF, Z_OFF, F_OFF = 0, 1024, 4096, 7168, 9216
M_ROWS = 9216 + 8 * 64
GU = 4
NG = (RB // BQ) * H // GU


def _tables():
    n = np.arange(128)[None, :]
    fs = []
    for kap in range(2):
        rows = []
        for e in range(NCH):
            k = (2 * (CR * e + np.arange(CR)) + kap)[:, None]
            th = 2.0 * np.pi * (k + 0.5) * n / 256.0
            rows += [np.cos(th), -np.sin(th)]
        fs.append(np.concatenate(rows, axis=0))
    f = np.stack(fs)
    finv = np.transpose(f, (0, 2, 1)) / 128.0
    r = np.arange(16)[:, None]
    a = np.arange(128)[None, :]
    sig, alo = a // 16, a % 16
    lo = np.zeros((2, 128, 128), np.float32)
    for rho in range(8):
        first = sig <= rho
        valid = np.where(sig < rho, True,
                 np.where(sig == rho, r > alo,
                  np.where(sig == rho + 1, r <= alo, True)))
        lo[1, 16 * rho:16 * rho + 16] = np.where(valid, 0.0, -BIG)
        lo[0, 16 * rho:16 * rho + 16] = np.where(valid & ~first, 0.0, -BIG)
    hi = np.where((sig > 0) | (r <= alo), 0.0, -BIG).astype(np.float32)
    return (jnp.asarray(f, jnp.bfloat16), jnp.asarray(finv, jnp.bfloat16),
            jnp.asarray(lo), jnp.asarray(hi))


def _tree(op, xs, ways=4):
    accs = []
    for i, x in enumerate(xs):
        if i < ways:
            accs.append(x)
        else:
            accs[i % ways] = op(accs[i % ways], x)
    while len(accs) > 1:
        accs = [op(accs[i], accs[i + 1]) if i + 1 < len(accs) else accs[i] for i in range(0, len(accs), 2)]
    return accs[0]


def _rows8(x):
    return [x[8 * i:8 * i + 8] for i in range(x.shape[0] // 8)]


def _kernel(q_ref, k_ref, v_ref, shk_ref, ssmk_ref, ssmd_ref, x_ref, wqkv_ref, wo_ref,
            f_ref, finv_ref, blo_ref, bhi_ref, out_hbm,
            wT_sc, wk_sc, wo_sc, fp_sc, xp_sc, rep_sc, vT_sc, m_sc, oT_sc, kv_sc, kpad_sc, y_sc,
            outa_sc, outb_sc, s_sc0, s_sc1, sems):
    s_scs = (s_sc0, s_sc1)
    j = pl.program_id(0)
    kap = j % 2
    c = j // 2
    f32, bf16, u32 = jnp.float32, jnp.bfloat16, jnp.uint32
    dz = lax.shift_right_logical(j, 10)

    def b_copy(step):
        return pltpu.make_async_copy(
            outb_sc.at[step % 2], out_hbm.at[0, pl.ds(step * RB, RB), pl.ds(D, D)], sems.at[step % 2])

    def a_copy(cc):
        return pltpu.make_async_copy(
            outa_sc.at[cc % 2], out_hbm.at[0, :, pl.ds(cc * 128, 128)], sems.at[2 + cc % 2])

    @pl.when(j > 0)
    def _():
        b_copy(j - 1).wait()

    @pl.when(jnp.logical_and(kap == 1, c > 0))
    def _():
        a_copy(c - 1).wait()

    @pl.when(j == 0)
    def _init():
        for t in range(4):
            wq = wqkv_ref[:, 128 * t:128 * t + 128].astype(f32)
            wT_sc[64 * t:64 * t + 64, :] = pltpu.bitcast(wq.T.astype(bf16), u32)
            wv = wqkv_ref[:, 2 * D + 128 * t:2 * D + 128 * t + 128].astype(f32)
            wT_sc[D // 2 + 64 * t:D // 2 + 64 * t + 64, :] = pltpu.bitcast(wv.T.astype(bf16), u32)
        wk_sc[...] = pltpu.bitcast(wqkv_ref[:, D:2 * D], u32)
        wo_sc[...] = pltpu.bitcast(wo_ref[...], u32)
        for t in range(2):
            fp_sc[t] = pltpu.bitcast(f_ref[t], u32)
            fp_sc[2 + t] = pltpu.bitcast(finv_ref[t], u32)
        rep_sc[:, 0:128, :] = jnp.zeros((H, 128, 128), u32)
        vT_sc[:, 0:256] = jnp.zeros((D, 256), bf16)
        kpad_sc[0:8, :] = jnp.zeros((8, 128), f32)

    @pl.when(kap == 0)
    def _kv():
        kpad_sc[8:, :] = k_ref[...].astype(f32)
        taps = shk_ref[...].astype(f32).T
        for s in range(NB):
            acc = kpad_sc[8 + 128 * s:8 + 128 * s + 128, :] * taps[0:1, :]
            for tau in range(1, 4):
                acc = acc + kpad_sc[8 + 128 * s - tau:8 + 128 * s - tau + 128, :] * taps[tau:tau + 1, :]
            kvb = (acc * v_ref[128 * s:128 * s + 128, :].astype(f32)).astype(bf16)
            kv_sc[64 * s:64 * s + 64, :] = pltpu.bitcast(kvb, u32)

    sg = jnp.where(kap == 0, 1.0, -1.0).astype(f32)
    zero = lambda sh: pl.multiple_of(lax.shift_right_logical(j, sh) * 8, 8)
    bq_, bu_, bz_, bf_ = zero(11), zero(12), zero(13), zero(14)
    mq = lambda r, n: (pl.ds(bq_ + Q_OFF + r, n), slice(None))
    mu = lambda r, n: (pl.ds(bu_ + U_OFF + r, n), slice(None))
    mg = lambda r, n: (pl.ds(bu_ + G_OFF + r, n), slice(None))
    mz = lambda r, n: (pl.ds(bz_ + Z_OFF + r, n), slice(None))
    fence_cnt = [0]

    def fence(val):
        m_sc[pl.ds(bf_ + F_OFF + 8 * fence_cnt[0], 8), :] = val
        fence_cnt[0] += 1

    def a_fwd():
        fk = pltpu.bitcast(fp_sc[kap], bf16)
        hprev = None
        for s in range(NB):
            hh = lax.dot_general(fk, ssmk_ref[:, 128 * s:128 * s + 128], (((1,), (1,)), ((), ())),
                                 preferred_element_type=f32)
            if hprev is None:
                gr, gi = hh[0:64], hh[64:128]
            else:
                gr = hh[0:64] - sg * hprev[64:128]
                gi = hh[64:128] + sg * hprev[0:64]
            m_sc[mg(192 * s, 64)] = gr
            m_sc[mg(192 * s + 64, 64)] = gi - gr
            m_sc[mg(192 * s + 128, 64)] = gr + gi
            hprev = hh
            kvt = pltpu.bitcast(kv_sc[64 * s:64 * s + 64, :], bf16)
            uu = jnp.dot(fk, kvt, preferred_element_type=f32)
            m_sc[mu(192 * s, 128)] = uu
            m_sc[mu(192 * s + 128, 64)] = uu[0:64] + uu[64:128]

    ZR = 16

    def zunit(a, ch):
        r0 = ZR * ch
        ldu = lambda s: tuple(m_sc[mu(192 * s + 64 * i + r0, ZR)] for i in range(3))
        ldg = lambda s: tuple(m_sc[mg(192 * s + 64 * i + r0, ZR)] for i in range(3))
        acc = [None, None]

        def mac(o, u, g):
            p = (g[0] * u[2], u[0] * g[1], u[1] * g[2])
            acc[o] = p if acc[o] is None else tuple(x + y for x, y in zip(acc[o], p))

        uhi = ldu(2 * a + 1)
        for dl in range(2 * a + 2):
            g = ldg(dl)
            mac(1, uhi, g)
            if dl <= 2 * a:
                ulo = ldu(2 * a - dl)
                mac(0, ulo, g)
                uhi = ulo
        for o in range(2):
            k1, k2, k3 = acc[o]
            m_sc[mz(128 * (2 * a + o) + r0, ZR)] = k1 - k3
            m_sc[mz(128 * (2 * a + o) + 64 + r0, ZR)] = k1 + k2

    zq = [(a, ch) for a in range(NB // 2 - 1, -1, -1) for ch in range(64 // ZR)]

    def zwork(budget):
        while zq:
            fit = [z for z in zq if 4 * z[0] + 3 <= budget]
            if not fit:
                break
            a, ch = fit[0]
            zq.remove((a, ch))
            zunit(a, ch)
            budget -= 4 * a + 3

    dd = ssmd_ref[...].astype(f32)
    aslot = c % 2

    def inverse(t1):
        rows = slice(128 * t1, 128 * t1 + 128)
        yy = (jnp.dot(pltpu.bitcast(fp_sc[2 + kap], bf16), m_sc[mz(128 * t1, 128)].astype(bf16), preferred_element_type=f32)
              + jnp.where(kap == 1, y_sc[rows, :], 0.0))
        y_sc[rows, :] = yy
        kvf = pltpu.bitcast(kv_sc[64 * t1:64 * t1 + 64, :], bf16).astype(f32)
        outa_sc[aslot, rows, :] = (q_ref[rows, :].astype(f32) * (yy + kvf * dd)).astype(bf16)

    xp_sc[pl.ds(bq_, RB // 2), :] = pltpu.bitcast(x_ref[...], u32)
    xb = lambda: pltpu.bitcast(xp_sc[pl.ds(bq_, RB // 2), :], bf16)
    lane = lax.broadcasted_iota(jnp.int32, (RB // 2, 128), 1)
    m64 = lane < 64
    m32 = (lane // 32) % 2 == 0
    m16 = (lane // 16) % 2 == 0

    def k_proj(g):
        kf = jnp.dot(xb(), pltpu.bitcast(wk_sc[:, 128 * g:128 * g + 128], bf16), preferred_element_type=f32)
        fence(kf[RB - 8:RB])
        kg = pltpu.bitcast(kf.astype(bf16), u32)
        row0 = pl.multiple_of(128 + (RB // 2) * j, 8)
        r = pltpu.roll(kg, 64, 1)
        lvl1 = [jnp.where(m64, kg, r), jnp.where(m64, r, kg)]
        lvl2 = []
        for a_ in lvl1:
            r = pltpu.roll(a_, 32, 1)
            lvl2 += [jnp.where(m32, a_, r), jnp.where(m32, r, a_)]
        hh_ = 0
        for b_ in lvl2:
            r = pltpu.roll(b_, 16, 1)
            for z in (jnp.where(m16, b_, r), jnp.where(m16, r, b_)):
                rep_sc[8 * g + hh_, pl.ds(row0, RB // 2), :] = z
                hh_ += 1

    def q_proj(t):
        qt = lax.dot_general(pltpu.bitcast(wT_sc[64 * t:64 * t + 64, :], bf16), xb(), (((1,), (1,)), ((), ())),
                             preferred_element_type=f32) * QSCALE
        for b in range(RB // BQ):
            m_sc[mq(D * b + 128 * t, 128)] = qt[:, BQ * b:BQ * b + BQ]

    def v_proj(t):
        vt = lax.dot_general(pltpu.bitcast(wT_sc[D // 2 + 64 * t:D // 2 + 64 * t + 64, :], bf16), xb(), (((1,), (1,)), ((), ())),
                             preferred_element_type=f32)
        fence(vt[120:128, 128:256])
        vT_sc[128 * t:128 * t + 128, pl.ds(pl.multiple_of(256 + RB * j, 128), RB)] = vt.astype(bf16)

    slot16 = lax.broadcasted_iota(jnp.int32, (16, 128), 1) // 16
    rho56 = lax.broadcasted_iota(jnp.int32, (56, 128), 0) // 8
    slot56 = lax.broadcasted_iota(jnp.int32, (56, 128), 1) // 16
    first56 = slot56 <= rho56
    rho112 = lax.broadcasted_iota(jnp.int32, (112, 128), 0) // 16
    slot112 = lax.broadcasted_iota(jnp.int32, (112, 128), 1) // 16
    first112 = slot112 <= rho112
    jmin = jnp.minimum(j, 1)
    midb0 = jnp.where(j == 0, -BIG, 0.0).astype(f32)

    def qk(n):
        ms = []
        sc = s_scs[n % 2]
        for uu in range(GU):
            un = n * GU + uu
            b, h = un // H, un % H
            base = pl.multiple_of((RB // 2) * j + 64 * b, 8)
            qh = m_sc[mq(D * b + 16 * h, 16)]
            wq = jnp.concatenate([jnp.where(slot16 == sgm, qh, 0.0) for sgm in range(8)], axis=0).astype(bf16)
            lhs_m = jnp.where(first56, rep_sc[h, pl.ds(base, 56), :], rep_sc[h, pl.ds(base + 136, 56), :])
            lhs = pltpu.bitcast(jnp.concatenate([lhs_m, rep_sc[h, pl.ds(base + 56, 80), :]], axis=0), bf16)
            st = jnp.dot(lhs, wq, preferred_element_type=f32)
            s_lo = st[0:128] + blo_ref[jmin]
            s_mid = st[128:256]
            s_hi = st[256:272] + bhi_ref[...]
            mm = _tree(jnp.maximum, _rows8(s_mid), 2)
            if b == 0:
                mm = mm + midb0
            m8 = jnp.maximum(_tree(jnp.maximum, _rows8(s_lo) + _rows8(s_hi), 2), mm)
            ms.append(jnp.max(m8, axis=0, keepdims=True))
            sc[dz + uu, 0:128, :] = s_lo
            sc[dz + uu, 128:256, :] = s_mid
            sc[dz + uu, 256:272, :] = s_hi
        return ms

    def softmax_pv(n, ms):
        sc = s_scs[n % 2]
        for uu in range(GU):
            un = n * GU + uu
            b, h = un // H, un % H
            col0 = pl.multiple_of(RB * j + BQ * b, 128)
            m = ms[uu]
            p_lo = jnp.exp2(sc[dz + uu, 0:128, :] - m)
            p_mid = jnp.exp2(sc[dz + uu, 128:256, :] - ((m - midb0) if b == 0 else m))
            p_hi = jnp.exp2(sc[dz + uu, 256:272, :] - m)
            l = jnp.sum(_tree(jnp.add, _rows8(p_lo) + _rows8(p_mid) + _rows8(p_hi), 4), axis=0, keepdims=True)
            frame = jnp.concatenate([
                jnp.where(first112, p_lo[0:112], 0.0), p_lo[112:128], p_mid, p_hi,
                jnp.where(first112, 0.0, p_lo[0:112])], axis=0).astype(bf16)
            vh = vT_sc[16 * h:16 * h + 16, pl.ds(col0, 384)]
            ot = jnp.dot(vh, frame, preferred_element_type=f32)
            oT_sc[dz + b, 16 * h:16 * h + 16, :] = ot * (1.0 / l)

    def outproj(b):
        o = oT_sc[dz + b].T.astype(bf16)
        outb_sc[j % 2, BQ * b:BQ * b + BQ, :] = jnp.dot(o, pltpu.bitcast(wo_sc[...], bf16), preferred_element_type=f32).astype(bf16)

    ZP, ZA = 31, 16
    a_fwd()
    for g in range(4):
        k_proj(g)
        zwork(ZP)
    for t in range(4):
        q_proj(t)
        zwork(ZP)
    for t in range(4):
        v_proj(t)
        if t < 2:
            zwork(ZP)
    ms = qk(0)
    for n in range(NG):
        ms_next = qk(n + 1) if n + 1 < NG else None
        zwork(ZA)
        softmax_pv(n, ms)
        if n == NG // 2 + 2:
            outproj(0)
        ms = ms_next
    zwork(10 ** 6)
    for t1 in range(NB):
        inverse(t1)
    outproj(1)

    b_copy(j).start()

    @pl.when(kap == 1)
    def _():
        a_copy(c).start()

    @pl.when(j == NSTEP - 1)
    def _fin():
        b_copy(j).wait()
        a_copy(c).wait()


@jax.jit
def pallas_concat_heads__ssm_conv_h3__sliding_block__prompt_kernel(
    A_q, A_k, A_v, A_shift_k, A_ssm_k, A_ssm_D, B_x, B_wqkv, B_wo):
    f, finv, blo, bhi = _tables()
    strip = pl.BlockSpec((None, S, 128), lambda j: (0, 0, j // 2))
    full = lambda shape: pl.BlockSpec(shape, lambda j: (0,) * len(shape))
    in_specs = [
        strip, strip, strip,
        pl.BlockSpec((128, 4), lambda j: (j // 2, 0)),
        pl.BlockSpec((128, S), lambda j: (j // 2, 0)),
        pl.BlockSpec((1, 128), lambda j: (0, j // 2)),
        pl.BlockSpec((None, RB, D), lambda j: (0, j, 0)),
        full((D, 3 * D)), full((D, D)),
        full((2, 128, 128)), full((2, 128, 128)), full((2, 128, 128)), full((16, 128)),
    ]
    scratch = [
        pltpu.VMEM((D, D), jnp.uint32),
        pltpu.VMEM((D // 2, D), jnp.uint32),
        pltpu.VMEM((D // 2, D), jnp.uint32),
        pltpu.VMEM((4, 64, 128), jnp.uint32),
        pltpu.VMEM((RB // 2, D), jnp.uint32),
        pltpu.VMEM((H, (S + 256) // 2, 128), jnp.uint32),
        pltpu.VMEM((D, S + 256), jnp.bfloat16),
        pltpu.VMEM((M_ROWS, 128), jnp.float32),
        pltpu.VMEM((RB // BQ, D, BQ), jnp.float32),
        pltpu.VMEM((S // 2, 128), jnp.uint32),
        pltpu.VMEM((S + 8, 128), jnp.float32),
        pltpu.VMEM((S, 128), jnp.float32),
        pltpu.VMEM((2, S, 128), jnp.bfloat16),
        pltpu.VMEM((2, RB, D), jnp.bfloat16),
        pltpu.VMEM((GU, 272, 128), jnp.float32),
        pltpu.VMEM((GU, 272, 128), jnp.float32),
        pltpu.SemaphoreType.DMA((4,)),
    ]
    return pl.pallas_call(
        _kernel,
        grid=(NSTEP,),
        in_specs=in_specs,
        out_specs=pl.BlockSpec(memory_space=pl.ANY),
        out_shape=jax.ShapeDtypeStruct((1, S, 2 * D), jnp.bfloat16),
        scratch_shapes=scratch,
        compiler_params=pltpu.CompilerParams(
            dimension_semantics=("arbitrary",),
            vmem_limit_bytes=100 * 1024 * 1024),
    )(A_q, A_k, A_v, A_shift_k, A_ssm_k, A_ssm_D.reshape(1, D), B_x, B_wqkv, B_wo, f, finv, blo, bhi)
```

```python
import math
import numpy as np
import jax
import jax.numpy as jnp
from jax import lax
import jax.experimental.pallas as pl
import jax.experimental.pallas.tpu as pltpu

S = 2048
D = 512
H = 32
DH = 16
BQ = 128
RB = 512
NQ = RB // BQ
NSTEP = S // RB
NB = S // 128
NC = D // 128
BIG = 1e30
QSCALE = (DH ** -0.5) * math.log2(math.e)
NU = NQ * H
LAG = 3
CS, BS = 72, 232
UG = 32 * BS
Z_OFF = 2 * UG
M_ROWS = Z_OFF + 4096
ZF = 12
ZR = 16
(SEM_Q, SEM_K, SEM_V, SEM_S, SEM_X) = (0, 4, 8, 12, 16)
(SEM_W, SEM_WK, SEM_WO, SEM_F, SEM_BLO, SEM_BHI, SEM_SHK, SEM_D, SEM_OB, SEM_OA) = range(20, 30)
NSEM = 30


def _tables():
    n = np.arange(128)[None, :]
    fs = []
    for kap in range(2):
        k = (2 * np.arange(64) + kap)[:, None]
        th = 2.0 * np.pi * (k + 0.5) * n / 256.0
        fs.append(np.concatenate([np.cos(th), -np.sin(th)], axis=0))
    f = np.stack(fs)
    finv = np.transpose(f, (0, 2, 1)) / 128.0
    r = np.arange(16)[:, None]
    a = np.arange(128)[None, :]
    sig, alo = a // 16, a % 16
    lo = np.zeros((2, 128, 128), np.float32)
    for rho in range(8):
        first = sig <= rho
        valid = np.where(sig < rho, True,
                 np.where(sig == rho, r > alo,
                  np.where(sig == rho + 1, r <= alo, True)))
        lo[1, 16 * rho:16 * rho + 16] = np.where(valid, 0.0, -BIG)
        lo[0, 16 * rho:16 * rho + 16] = np.where(valid & ~first, 0.0, -BIG)
    hi = np.where((sig > 0) | (r <= alo), 0.0, -BIG).astype(np.float32)
    return (jnp.asarray(np.concatenate([f, finv]), jnp.bfloat16), jnp.asarray(lo), jnp.asarray(hi))


def _tree(op, xs, ways=4):
    accs = []
    for i, x in enumerate(xs):
        if i < ways:
            accs.append(x)
        else:
            accs[i % ways] = op(accs[i % ways], x)
    while len(accs) > 1:
        accs = [op(accs[i], accs[i + 1]) if i + 1 < len(accs) else accs[i] for i in range(0, len(accs), 2)]
    return accs[0]


def _rows8(x):
    return [x[8 * i:8 * i + 8] for i in range(x.shape[0] // 8)]


def _kernel(q_hbm, k_hbm, v_hbm, shk_hbm, ssmk_hbm, ssmd_hbm, x_hbm, wqkv_hbm, wo_hbm,
            f_hbm, blo_hbm, bhi_hbm, out_hbm,
            q_in, k_in, v_in, shk_in, ssmk_in, d_in, x_in, wqv_in, wk_in, wo_in, fp_sc, blo_ref, bhi_ref,
            wT_sc, par_sc, kst_sc, rep_sc, vT_sc, qT_sc, m_sc, oT_sc, kv_sc,
            outa_sc, outb_sc, sems):
    j = pl.program_id(0)
    c = j
    f32, bf16, u32 = jnp.float32, jnp.bfloat16, jnp.uint32
    NT = (((1,), (1,)), ((), ()))
    zero = lambda sh: pl.multiple_of(lax.shift_right_logical(j, sh) * 8, 8)
    bu_, bz_ = zero(12), zero(13)
    mu = lambda kap, r, n: (pl.ds(bu_ + UG * kap + r, n), slice(None))
    mg = lambda kap, r, n: (pl.ds(bu_ + UG * kap + 16 * BS + r, n), slice(None))
    mz = lambda r, n: (pl.ds(bz_ + Z_OFF + r, n), slice(None))
    rrow = pl.multiple_of((RB // 2) * j, 128)
    packed = lambda ref, idx: pltpu.bitcast(ref.bitcast(u32)[idx], bf16)

    def tiles_copy(src, dst, sem, n):
        return [pltpu.make_async_copy(src.at[:, pl.ds(128 * t, 128)], dst.at[t], sems.at[sem]) for t in range(n)]

    def strip_copy(src, dst, sem0, cc):
        return [pltpu.make_async_copy(src.at[0, :, pl.ds(cc * 128, 128)], dst.at[cc], sems.at[sem0 + cc])]

    q_copy = lambda cc: strip_copy(q_hbm, q_in, SEM_Q, cc)
    k_copy = lambda cc: strip_copy(k_hbm, k_in, SEM_K, cc)
    v_copy = lambda cc: strip_copy(v_hbm, v_in, SEM_V, cc)
    s_copy = lambda cc: tiles_copy(ssmk_hbm.at[pl.ds(cc * 128, 128), :], ssmk_in.at[cc], SEM_S + cc, NB)
    x_copy = lambda st: tiles_copy(x_hbm.at[0, pl.ds(st * RB, RB), :], x_in.at[st], SEM_X + st, 4)
    whole = lambda src, dst, sem: [pltpu.make_async_copy(src, dst, sems.at[sem])]
    w_copy = (tiles_copy(wqkv_hbm.at[:, pl.ds(0, D)], wqv_in.at[0], SEM_W, 4)
              + tiles_copy(wqkv_hbm.at[:, pl.ds(2 * D, D)], wqv_in.at[1], SEM_W, 4))
    wk_copy = tiles_copy(wqkv_hbm.at[:, pl.ds(D, D)], wk_in, SEM_WK, 4)
    wo_copy = tiles_copy(wo_hbm, wo_in, SEM_WO, 4)
    small = (whole(f_hbm, fp_sc, SEM_F) + whole(shk_hbm, shk_in, SEM_SHK) + whole(ssmd_hbm, d_in, SEM_D)
             + whole(blo_hbm, blo_ref, SEM_BLO) + whole(bhi_hbm, bhi_ref, SEM_BHI))

    def start(cps):
        for cp in cps:
            cp.start()

    def wait(cps):
        for cp in cps:
            cp.wait()

    def b_copy(step):
        return pltpu.make_async_copy(
            outb_sc, out_hbm.at[0, pl.ds(step * RB, RB), pl.ds(D, D)], sems.at[SEM_OB])

    def a_copy(cc):
        return pltpu.make_async_copy(
            outa_sc, out_hbm.at[0, :, pl.ds(cc * 128, 128)], sems.at[SEM_OA])

    def outproj(b):
        o = oT_sc[b].T.astype(bf16)
        for nt in range(4):
            r = jnp.dot(o, packed(wo_in, nt), preferred_element_type=f32)
            outb_sc[BQ * b:BQ * b + BQ, 128 * nt:128 * nt + 128] = r.astype(bf16)

    def init_weights():
        for w in range(2):
            for t in range(4):
                wt = wqv_in[w, t].astype(f32).T.astype(bf16)
                for kt in range(4):
                    wT_sc[kt, D * w + 128 * t:D * w + 128 * t + 128, :] = wt[:, 128 * kt:128 * kt + 128]

    def pphase(first):
        lane = lax.broadcasted_iota(jnp.int32, (BQ, 128), 1)
        l16 = lane % 16

        def kv_piece(s):
            taps = par_sc[c]
            kf = k_in[c, 128 * s:128 * s + 128, :].astype(f32)
            if s == 0:
                prev = jnp.zeros((8, 128), f32)
            else:
                prev = k_in[c, 128 * s - 16:128 * s, :].astype(f32)[8:16]
            ext = jnp.concatenate([prev, kf], axis=0)
            acc = kf * taps[0:1, :]
            for tau in range(1, 4):
                acc = acc + pltpu.roll(ext, tau, 0)[8:136] * taps[tau:tau + 1, :]
            kv_sc[128 * s:128 * s + 128, :] = (acc * v_in[c, 128 * s:128 * s + 128, :].astype(f32)).astype(bf16)

        kvp = lambda s: packed(kv_sc, (slice(64 * s, 64 * s + 64), slice(None)))
        ffwd = lambda: pltpu.bitcast(fp_sc.bitcast(u32)[0:2].reshape(128, 128), bf16)
        hprev = [None]

        def g_piece(s):
            hh = lax.dot_general(ffwd(), packed(ssmk_in, (c, s)), NT, preferred_element_type=f32)
            hp = hprev[0]
            for kap in range(2):
                hr, hi = hh[128 * kap:128 * kap + 64], hh[128 * kap + 64:128 * kap + 128]
                if hp is None:
                    gr, gi = hr, hi
                else:
                    pr, pi_ = hp[128 * kap:128 * kap + 64], hp[128 * kap + 64:128 * kap + 128]
                    gr, gi = (hr - pi_, hi + pr) if kap == 0 else (hr + pi_, hi - pr)
                m_sc[mg(kap, BS * s, 64)] = gr
                m_sc[mg(kap, BS * s + CS, 64)] = gi - gr
                m_sc[mg(kap, BS * s + 2 * CS, 64)] = gr + gi
            hprev[0] = hh

        def u_piece(s):
            kv_piece(s)
            uu = jnp.dot(ffwd(), kvp(s), preferred_element_type=f32)
            for kap in range(2):
                ur, ui = uu[128 * kap:128 * kap + 64], uu[128 * kap + 64:128 * kap + 128]
                m_sc[mu(kap, BS * s, 64)] = ur
                m_sc[mu(kap, BS * s + CS, 64)] = ui
                m_sc[mu(kap, BS * s + 2 * CS, 64)] = ur + ui

        def zunit(kap, a, ch):
            r0 = ZR * ch
            ldu = lambda s: tuple(m_sc[mu(kap, BS * s + CS * i + r0, ZR)] for i in range(3))
            ldg = lambda s: tuple(m_sc[mg(kap, BS * s + CS * i + r0, ZR)] for i in range(3))
            acc = [None, None]

            def mac(o, u, g):
                p = (g[0] * u[2], u[0] * g[1], u[1] * g[2])
                acc[o] = p if acc[o] is None else tuple(x + y for x, y in zip(acc[o], p))

            uhi = ldu(2 * a + 1)
            for dl in range(2 * a + 2):
                g = ldg(dl)
                mac(1, uhi, g)
                if dl <= 2 * a:
                    ulo = ldu(2 * a - dl)
                    mac(0, ulo, g)
                    uhi = ulo
            for o in range(2):
                k1, k2, k3 = acc[o]
                m_sc[mz(256 * (2 * a + o) + 128 * kap + r0, ZR)] = k1 - k3
                m_sc[mz(256 * (2 * a + o) + 128 * kap + 64 + r0, ZR)] = k1 + k2

        zq = [(kap, a, ch) for a in range(NB // 2 - 1, -1, -1) for kap in range(2) for ch in range(64 // ZR)]

        def zall(n=10 ** 6):
            for _ in range(min(n, len(zq))):
                zunit(*zq.pop(0))

        def inverse(t1):
            rows = slice(128 * t1, 128 * t1 + 128)
            finv = jnp.concatenate([packed(fp_sc, 2), packed(fp_sc, 3)], axis=1)
            yy = jnp.dot(finv, m_sc[mz(256 * t1, 256)].astype(bf16), preferred_element_type=f32)
            dd = par_sc[c, 4:5, :]
            outa_sc[rows, :] = (q_in[c, rows, :].astype(f32) * (yy + kvp(t1).astype(f32) * dd)).astype(bf16)

        def xrows(hf):
            return jnp.concatenate(
                [packed(x_in, (j, kt, slice(128 * hf, 128 * hf + 128), slice(None))) for kt in range(4)], axis=1)

        def wtrows(r0):
            return jnp.concatenate(
                [packed(wT_sc, (kt, slice(r0 // 2, r0 // 2 + 64), slice(None))) for kt in range(4)], axis=1)

        def k_proj(g, hf):
            kf = jnp.dot(xrows(hf), packed(wk_in, g), preferred_element_type=f32)
            kst_sc[2 * g + hf] = kf.astype(bf16)
            kg = kst_sc.bitcast(u32)[2 * g + hf]
            dst = pl.ds(rrow + 128 + 128 * hf, 128)
            for hl in range(8):
                rep_sc[8 * g + hl, dst, :] = jnp.take_along_axis(kg, l16 + 16 * hl, axis=1)

        def q_proj(t, hf):
            qt = lax.dot_general(wtrows(128 * t), xrows(hf), NT, preferred_element_type=f32) * QSCALE
            for b in range(2):
                qT_sc[2 * hf + b, 128 * t:128 * t + 128, :] = qt[:, BQ * b:BQ * b + BQ]

        def v_proj(t, hf):
            vt = lax.dot_general(wtrows(D + 128 * t), xrows(hf), NT, preferred_element_type=f32).astype(bf16)
            for b in range(2):
                vT_sc[2 + NQ * j + 2 * hf + b, 128 * t:128 * t + 128, :] = vt[:, BQ * b:BQ * b + BQ]

        if not first:
            outproj(0)
            outproj(1)
        if first:
            for s in range(NB):
                g_piece(s)
            wait(k_copy(0) + v_copy(0))
            for s in range(NB):
                u_piece(s)
        else:
            for s in range(NB):
                g_piece(s)
                u_piece(s)
        if first:
            zall(ZF)
            wait(w_copy + wk_copy + x_copy(0))
            start(q_copy(0) + wo_copy)
            for cc in range(1, NC):
                start(k_copy(cc) + v_copy(cc) + s_copy(cc) + x_copy(cc) + q_copy(cc))
            init_weights()
        else:
            outproj(2)
        zall()
        for hf in range(2):
            for g in range(4):
                k_proj(g, hf)
        for hf in range(2):
            for t in range(4):
                q_proj(t, hf)
        for hf in range(2):
            for t in range(4):
                v_proj(t, hf)
        if first:
            wait(q_copy(0))
        else:
            outproj(3)
            b_copy(j - 1).start()
        for t1 in range(NB):
            inverse(t1)
        a_copy(c).start()

    @pl.when(j == 0)
    def _():
        start(small + s_copy(0) + k_copy(0) + v_copy(0))
        wait(small)
        shk = shk_in[...].astype(f32)
        dvec = d_in[...].astype(f32).reshape(1, D)
        for cc in range(NC):
            par_sc[cc] = jnp.concatenate(
                [shk[:, 128 * cc:128 * cc + 128], dvec[:, 128 * cc:128 * cc + 128], jnp.zeros((3, 128), f32)], axis=0)
        wait(s_copy(0))
        start(wk_copy + x_copy(0) + w_copy)
        pphase(True)

    @pl.when(j == 1)
    def _():
        wait(wo_copy)

    @pl.when(j > 1)
    def _():
        b_copy(j - 2).wait()

    @pl.when(j > 0)
    def _():
        wait(k_copy(c) + v_copy(c) + s_copy(c) + x_copy(c) + q_copy(c))
        a_copy(c - 1).wait()
        pphase(False)

    slot16 = lax.broadcasted_iota(jnp.int32, (16, 128), 1) // 16
    rho56 = lax.broadcasted_iota(jnp.int32, (56, 128), 0) // 8
    slot56 = lax.broadcasted_iota(jnp.int32, (56, 128), 1) // 16
    first56 = slot56 <= rho56
    rho112 = lax.broadcasted_iota(jnp.int32, (112, 128), 0) // 16
    slot112 = lax.broadcasted_iota(jnp.int32, (112, 128), 1) // 16
    first112 = slot112 <= rho112

    zf = lax.shift_right_logical(j, 20).astype(f32)

    def tphase(first):
        def qk(un):
            b, h = un // H, un % H
            head = first and b < 2
            base = rrow + 64 * b
            qh = qT_sc[b, 16 * h:16 * h + 16, :]
            wq = jnp.concatenate([jnp.where(slot16 == sgm, qh, 0.0) for sgm in range(8)], axis=0).astype(bf16)
            last = rep_sc[h, pl.ds(base + 136, 56), :]
            if not head:
                lhs_u = jnp.concatenate([jnp.where(first56, rep_sc[h, pl.ds(base, 56), :], last),
                                         rep_sc[h, pl.ds(base + 56, 80), :]], axis=0)
                spl = (0, 80, 144, 208, 272)
            elif b == 0:
                lhs_u = jnp.concatenate([last, rep_sc[h, pl.ds(base + 128, 8), :]], axis=0)
                spl = (0, 32, 64, 96, 128)
            else:
                lhs_u = jnp.concatenate([last, rep_sc[h, pl.ds(base + 64, 72), :]], axis=0)
                spl = (0, 64, 128, 192, 256)
            return jnp.concatenate([
                jnp.dot(pltpu.bitcast(lhs_u[spl[i] // 2:spl[i + 1] // 2], bf16), wq, preferred_element_type=f32)
                for i in range(4)], axis=0)

        def softmax(un, st):
            b = un // H
            head = first and b < 2
            nlo = 112 if head else 128
            nmid = 0 if (head and b == 0) else 128
            s_lo = st[0:nlo] + (blo_ref[0, 0:112, :] if head else blo_ref[1])
            s_hi = st[nlo + nmid:nlo + nmid + 16] + bhi_ref[...]
            m8 = _tree(jnp.maximum, _rows8(s_lo) + _rows8(s_hi), 2)
            if nmid:
                s_mid = st[nlo:nlo + nmid]
                m8 = jnp.maximum(m8, _tree(jnp.maximum, _rows8(s_mid), 2))
            m = jnp.max(m8, axis=0, keepdims=True)
            p_lo = jnp.exp2(s_lo - m)
            p_hi = jnp.exp2(s_hi - m)
            mid = [jnp.exp2(s_mid - (m - zf))] if nmid else []
            rows = _rows8(p_lo) + (_rows8(mid[0]) if nmid else []) + _rows8(p_hi)
            l = jnp.sum(_tree(jnp.add, rows, 4), axis=0, keepdims=True)
            if head:
                parts = mid + [p_hi, p_lo]
            else:
                parts = [jnp.where(first112, p_lo[0:112], 0.0), p_lo[112:128]] + mid + [
                    p_hi, jnp.where(first112, 0.0, p_lo[0:112])]
            return jnp.concatenate(parts, axis=0).astype(bf16), l

        def pv(un, frame, l):
            b, h = un // H, un % H
            nt = frame.shape[0] // 128
            vh = jnp.concatenate(
                [packed(vT_sc, (NQ * j + b + i, slice(8 * h, 8 * h + 8), slice(None))) for i in range(3 - nt, 3)],
                axis=1)
            ot = jnp.dot(vh, frame, preferred_element_type=f32)
            oT_sc[b, 16 * h:16 * h + 16, :] = ot * (1.0 / l)

        fr = {}
        pend = list(range(NU))
        for n in range(NU):
            fr[n] = softmax(n, qk(n))
            lag = 2 * LAG if (first and n < H) else LAG
            while pend[0] <= n - lag:
                pv(pend[0], *fr.pop(pend[0]))
                pend.pop(0)
        for u in pend:
            pv(u, *fr.pop(u))

    @pl.when(j == 0)
    def _():
        tphase(True)

    @pl.when(j > 0)
    def _():
        tphase(False)

    @pl.when(j == NSTEP - 1)
    def _fin():
        b_copy(j - 1).wait()
        last = [pltpu.make_async_copy(
            outb_sc.at[pl.ds(BQ * b, BQ), :],
            out_hbm.at[0, pl.ds((NSTEP - 1) * RB + BQ * b, BQ), pl.ds(D, D)], sems.at[SEM_X + b]) for b in range(NQ)]
        for b in range(NQ):
            outproj(b)
            last[b].start()
        a_copy(c).wait()
        wait(last)


@jax.jit
def pallas_concat_heads__ssm_conv_h3__sliding_block__prompt_kernel(
    A_q, A_k, A_v, A_shift_k, A_ssm_k, A_ssm_D, B_x, B_wqkv, B_wo):
    f, blo, bhi = _tables()
    bf16, f32, u32 = jnp.bfloat16, jnp.float32, jnp.uint32
    scratch = [
        pltpu.VMEM((NC, S, 128), bf16),
        pltpu.VMEM((NC, S, 128), bf16),
        pltpu.VMEM((NC, S, 128), bf16),
        pltpu.VMEM((4, D), bf16),
        pltpu.VMEM((NC, NB, 128, 128), bf16),
        pltpu.VMEM((D,), bf16),
        pltpu.VMEM((NSTEP, 4, RB, 128), bf16),
        pltpu.VMEM((2, 4, D, 128), bf16),
        pltpu.VMEM((4, D, 128), bf16),
        pltpu.VMEM((4, D, 128), bf16),
        pltpu.VMEM((4, 128, 128), bf16),
        pltpu.VMEM((2, 128, 128), f32),
        pltpu.VMEM((16, 128), f32),
        pltpu.VMEM((4, 2 * D, 128), bf16),
        pltpu.VMEM((NC, 8, 128), f32),
        pltpu.VMEM((8, 256, 128), bf16),
        pltpu.VMEM((H, (S + 256) // 2, 128), u32),
        pltpu.VMEM((NB + 2, D, 128), bf16),
        pltpu.VMEM((NQ, D, 128), f32),
        pltpu.VMEM((M_ROWS, 128), f32),
        pltpu.VMEM((NQ, D, BQ), f32),
        pltpu.VMEM((S, 128), bf16),
        pltpu.VMEM((S, 128), bf16),
        pltpu.VMEM((RB, D), bf16),
        pltpu.SemaphoreType.DMA((NSEM,)),
    ]
    return pl.pallas_call(
        _kernel,
        grid=(NSTEP,),
        in_specs=[pl.BlockSpec(memory_space=pl.ANY)] * 12,
        out_specs=pl.BlockSpec(memory_space=pl.ANY),
        out_shape=jax.ShapeDtypeStruct((1, S, 2 * D), bf16),
        scratch_shapes=scratch,
        compiler_params=pltpu.CompilerParams(
            dimension_semantics=("arbitrary",),
            vmem_limit_bytes=110 * 1024 * 1024),
    )(A_q, A_k, A_v, A_shift_k.T, A_ssm_k, A_ssm_D, B_x, B_wqkv, B_wo, f, blo, bhi)
```

```python
import math
import numpy as np
import jax
import jax.numpy as jnp
from jax import lax
import jax.experimental.pallas as pl
import jax.experimental.pallas.tpu as pltpu

S = 2048
D = 512
H = 32
DH = 16
BQ = 128
RB = 512
NQ = RB // BQ
NSTEP = S // RB
NB = S // 128
NC = D // 128
BIG = 1e30
QSCALE = (DH ** -0.5) * math.log2(math.e)
NU = NQ * H
LAG = 4
CS, BS = 72, 232
UG = 32 * BS
Z_OFF = 2 * UG
F_OFF = Z_OFF + 4096
M_ROWS = F_OFF + 16
ZR = 16
(SEM_Q, SEM_K, SEM_V, SEM_S, SEM_X) = (0, 4, 8, 12, 16)
(SEM_W, SEM_WK, SEM_WO, SEM_F, SEM_BLO, SEM_BHI, SEM_SHK, SEM_D, SEM_OB, SEM_OA) = range(20, 30)
NSEM = 31
ZH = (544, 1088)


def _tables():
    n = np.arange(128)[None, :]
    fs = []
    for kap in range(2):
        k = (2 * np.arange(64) + kap)[:, None]
        th = 2.0 * np.pi * (k + 0.5) * n / 256.0
        fs.append(np.concatenate([np.cos(th), -np.sin(th)], axis=0))
    f = np.stack(fs)
    finv = np.transpose(f, (0, 2, 1)) / 128.0
    r = np.arange(16)[:, None]
    a = np.arange(128)[None, :]
    sig, alo = a // 16, a % 16
    lo = np.zeros((2, 128, 128), np.float32)
    for rho in range(8):
        first = sig <= rho
        valid = np.where(sig < rho, True,
                 np.where(sig == rho, r > alo,
                  np.where(sig == rho + 1, r <= alo, True)))
        lo[1, 16 * rho:16 * rho + 16] = np.where(valid, 0.0, -BIG)
        lo[0, 16 * rho:16 * rho + 16] = np.where(valid & ~first, 0.0, -BIG)
    hi = np.where((sig > 0) | (r <= alo), 0.0, -BIG).astype(np.float32)
    return (jnp.asarray(np.concatenate([f, finv]), jnp.bfloat16), jnp.asarray(lo), jnp.asarray(hi))


def _tree(op, xs, ways=4):
    accs = []
    for i, x in enumerate(xs):
        if i < ways:
            accs.append(x)
        else:
            accs[i % ways] = op(accs[i % ways], x)
    while len(accs) > 1:
        accs = [op(accs[i], accs[i + 1]) if i + 1 < len(accs) else accs[i] for i in range(0, len(accs), 2)]
    return accs[0]


def _rows8(x):
    return [x[8 * i:8 * i + 8] for i in range(x.shape[0] // 8)]


def _kernel(q_hbm, k_hbm, v_hbm, shk_hbm, ssmk_hbm, ssmd_hbm, x_hbm, wqkv_hbm, wo_hbm,
            f_hbm, blo_hbm, bhi_hbm, out_hbm,
            q_in, k_in, v_in, shk_in, ssmk_in, d_in, x_in, wqv_in, wk_in, wo_in, fp_sc, blo_ref, bhi_ref,
            wT_sc, par_sc, kst_sc, rep_sc, vT_sc, qT_sc, m0_sc, m1_sc, oT_sc, kv_sc,
            outa_sc, outb_sc, sems):
    j = pl.program_id(0)
    ms = (m0_sc, m1_sc)
    f32, bf16, u32 = jnp.float32, jnp.bfloat16, jnp.uint32
    NT = (((1,), (1,)), ((), ()))
    zero = lambda sh: pl.multiple_of(lax.shift_right_logical(j, sh) * 8, 8)
    bz_, bf_ = zero(13), zero(14)
    mu = lambda kap, r, n: (pl.ds(UG * kap + r, n), slice(None))
    mg = lambda kap, r, n: (pl.ds(UG * kap + 16 * BS + r, n), slice(None))
    mz = lambda r, n: (pl.ds(bz_ + Z_OFF + r, n), slice(None))
    rrow = pl.multiple_of((RB // 2) * j, 128)
    packed = lambda ref, idx: pltpu.bitcast(ref.bitcast(u32)[idx], bf16)

    def tiles_copy(src, dst, sem, n):
        return [pltpu.make_async_copy(src.at[:, pl.ds(128 * t, 128)], dst.at[t], sems.at[sem]) for t in range(n)]

    slot = lambda cc: (0, 1, 2, 1)[cc]
    qslot = lambda cc: cc % 2

    def strip_copy(src, dst, sem0, cc, sl):
        return [pltpu.make_async_copy(src.at[0, :, pl.ds(cc * 128, 128)], dst.at[sl], sems.at[sem0 + cc])]

    q_copy = lambda cc: strip_copy(q_hbm, q_in, SEM_Q, cc, qslot(cc))
    k_copy = lambda cc: strip_copy(k_hbm, k_in, SEM_K, cc, slot(cc))
    v_copy = lambda cc: strip_copy(v_hbm, v_in, SEM_V, cc, slot(cc))
    s_copy = lambda cc: [pltpu.make_async_copy(
        ssmk_hbm.at[pl.ds(cc * 128, 128), :], ssmk_in.at[slot(cc)], sems.at[SEM_S + cc])]
    x_copy = lambda st: tiles_copy(x_hbm.at[0, pl.ds(st * RB, RB), :], x_in.at[slot(st)], SEM_X + st, 4)
    whole = lambda src, dst, sem: [pltpu.make_async_copy(src, dst, sems.at[sem])]
    w_copy = (tiles_copy(wqkv_hbm.at[:, pl.ds(0, D)], wqv_in.at[0], SEM_W, 4)
              + tiles_copy(wqkv_hbm.at[:, pl.ds(2 * D, D)], wqv_in.at[1], SEM_W, 4))
    wk_copy = tiles_copy(wqkv_hbm.at[:, pl.ds(D, D)], wk_in, SEM_WK, 4)
    wo_copy = tiles_copy(wo_hbm, wo_in, SEM_WO, 4)
    small = whole(f_hbm, fp_sc, SEM_F) + whole(shk_hbm, shk_in, SEM_SHK) + whole(ssmd_hbm, d_in, SEM_D)
    masks = whole(blo_hbm, blo_ref, SEM_BLO) + whole(bhi_hbm, bhi_ref, SEM_BHI)

    total = lambda buf, sem: [pltpu.make_async_copy(buf, buf, sems.at[sem])]
    s_wait = s_copy
    x_wait = lambda st: total(x_in.at[slot(st)], SEM_X + st)

    def start(cps):
        for cp in cps:
            cp.start()

    def wait(cps):
        for cp in cps:
            cp.wait()

    def b_copy(step):
        return pltpu.make_async_copy(
            outb_sc.at[step % 2], out_hbm.at[0, pl.ds(step * RB, RB), pl.ds(D, D)], sems.at[SEM_OB])

    def a_copy(cc, p):
        return pltpu.make_async_copy(
            outa_sc.at[p], out_hbm.at[0, :, pl.ds(cc * 128, 128)], sems.at[SEM_OA + p])

    ostat = [None]

    def outproj(b, step):
        o = oT_sc[b].T.astype(bf16)
        for nt in range(4):
            r = jnp.dot(o, packed(wo_in, nt), preferred_element_type=f32)
            osl = (step % 2) if isinstance(step, int) else ostat[0]
            outb_sc[osl, BQ * b:BQ * b + BQ, 128 * nt:128 * nt + 128] = r.astype(bf16)

    def init_weights():
        for w in range(2):
            for t in range(4):
                wt = wqv_in[w, t].astype(f32).T.astype(bf16)
                for kt in range(4):
                    wT_sc[kt, D * w + 128 * t:D * w + 128 * t + 128, :] = wt[:, 128 * kt:128 * kt + 128]

    def zlist(lo, hi):
        out, acc = [], 0
        for a_ in range(NB // 2 - 1, -1, -1):
            for kap in range(2):
                for ch in range(64 // ZR):
                    if lo <= acc < hi:
                        out.append((kap, a_, ch))
                    acc += 4 * a_ + 3
        return out

    jdyn = j

    def pphase(mode, par):
        j = {'first': 0, 'final': NSTEP - 1}.get(mode, 2 if par == 0 else jdyn)
        sl = slot(j) if isinstance(j, int) else 1
        ostat[0] = 0
        rrow = (RB // 2) * j if isinstance(j, int) else pl.multiple_of((RB // 2) * j, 128)
        lane = lax.broadcasted_iota(jnp.int32, (BQ, 128), 1)
        l16 = lane % 16
        kvp = lambda p, s: packed(kv_sc, (p, slice(64 * s, 64 * s + 64), slice(None)))
        ffwd = lambda: pltpu.bitcast(fp_sc.bitcast(u32)[0:2].reshape(128, 128), bf16)
        hprev = [None]

        def kv_piece(s):
            cc = j
            taps = par_sc[cc]
            kf = k_in[sl, 128 * s:128 * s + 128, :].astype(f32)
            if s == 0:
                prev = jnp.zeros((8, 128), f32)
            else:
                prev = k_in[sl, 128 * s - 16:128 * s, :].astype(f32)[8:16]
            ext = jnp.concatenate([prev, kf], axis=0)
            acc = kf * taps[0:1, :]
            for tau in range(1, 4):
                acc = acc + pltpu.roll(ext, tau, 0)[8:136] * taps[tau:tau + 1, :]
            kv_sc[par, 128 * s:128 * s + 128, :] = (
                acc * v_in[sl, 128 * s:128 * s + 128, :].astype(f32)).astype(bf16)

        def g_piece(s):
            cc, m_sc = j, ms[par]
            hh = lax.dot_general(ffwd(), ssmk_in[sl, :, 128 * s:128 * s + 128], NT, preferred_element_type=f32)
            hp = hprev[0]
            for kap in range(2):
                hr, hi = hh[128 * kap:128 * kap + 64], hh[128 * kap + 64:128 * kap + 128]
                if hp is None:
                    gr, gi = hr, hi
                else:
                    pr, pi_ = hp[128 * kap:128 * kap + 64], hp[128 * kap + 64:128 * kap + 128]
                    gr, gi = (hr - pi_, hi + pr) if kap == 0 else (hr + pi_, hi - pr)
                m_sc[mg(kap, BS * s, 64)] = gr
                m_sc[mg(kap, BS * s + CS, 64)] = gi - gr
                m_sc[mg(kap, BS * s + 2 * CS, 64)] = gr + gi
            hprev[0] = hh

        def u_piece(s):
            m_sc = ms[par]
            kv_piece(s)
            uu = jnp.dot(ffwd(), kvp(par, s), preferred_element_type=f32)
            for kap in range(2):
                ur, ui = uu[128 * kap:128 * kap + 64], uu[128 * kap + 64:128 * kap + 128]
                m_sc[mu(kap, BS * s, 64)] = ur
                m_sc[mu(kap, BS * s + CS, 64)] = ui
                m_sc[mu(kap, BS * s + 2 * CS, 64)] = ur + ui

        def zunit(p, kap, a, ch, link=False):
            m_sc = ms[p]
            r0 = ZR * ch
            ldu = lambda s: tuple(m_sc[mu(kap, BS * s + CS * i + r0, ZR)] for i in range(3))
            ldg = lambda s: tuple(m_sc[mg(kap, BS * s + CS * i + r0, ZR)] for i in range(3))
            acc = [None, None]

            def mac(o, u, g):
                p = (g[0] * u[2], u[0] * g[1], u[1] * g[2])
                acc[o] = p if acc[o] is None else tuple(x + y for x, y in zip(acc[o], p))

            uhi = ldu(2 * a + 1)
            for dl in range(2 * a + 2):
                g = ldg(dl)
                mac(1, uhi, g)
                if dl <= 2 * a:
                    ulo = ldu(2 * a - dl)
                    mac(0, ulo, g)
                    uhi = ulo
            for o in range(2):
                k1, k2, k3 = acc[o]
                m_sc[mz(256 * (2 * a + o) + 128 * kap + r0, ZR)] = k1 - k3
                m_sc[mz(256 * (2 * a + o) + 128 * kap + 64 + r0, ZR)] = k1 + k2
            if link:
                ms[1 - p][pl.ds(bf_ + F_OFF, ZR), :] = acc[1][0]

        def zrun(p, units):
            for i, z in enumerate(units):
                zunit(p, *z, link=(i == len(units) - 1))

        def inverse(p, cc, t1):
            rows = slice(128 * t1, 128 * t1 + 128)
            finv = jnp.concatenate([packed(fp_sc, 2), packed(fp_sc, 3)], axis=1)
            yy = jnp.dot(finv, ms[p][mz(256 * t1, 256)].astype(bf16), preferred_element_type=f32)
            dd = par_sc[cc, 4:5, :]
            outa_sc[p, rows, :] = (q_in[p, rows, :].astype(f32) * (yy + kvp(p, t1).astype(f32) * dd)).astype(bf16)

        def xrows(hf):
            return jnp.concatenate(
                [packed(x_in, (sl, kt, slice(128 * hf, 128 * hf + 128), slice(None))) for kt in range(4)], axis=1)

        def wtrows(r0):
            return jnp.concatenate(
                [packed(wT_sc, (kt, slice(r0 // 2, r0 // 2 + 64), slice(None))) for kt in range(4)], axis=1)

        def k_mm(g, hf):
            kf = jnp.dot(xrows(hf), packed(wk_in, g), preferred_element_type=f32)
            kst_sc[2 * g + hf] = kf.astype(bf16)

        def k_rep(g, hf):
            kg = kst_sc.bitcast(u32)[2 * g + hf]
            dst = pl.ds(rrow + 128 + 128 * hf, 128)
            for hl in range(8):
                rep_sc[8 * g + hl, dst, :] = jnp.take_along_axis(kg, l16 + 16 * hl, axis=1)

        def k_proj(mm=True, rep=True):
            for hf in range(2):
                for g in range(4):
                    if mm:
                        k_mm(g, hf)
                    if rep:
                        k_rep(g, hf)

        def q_proj():
            for hf in range(2):
                for t in range(4):
                    qt = lax.dot_general(wtrows(128 * t), xrows(hf), NT, preferred_element_type=f32) * QSCALE
                    for b in range(2):
                        qT_sc[2 * hf + b, 128 * t:128 * t + 128, :] = qt[:, BQ * b:BQ * b + BQ]

        def v_proj():
            for hf in range(2):
                for t in range(4):
                    vt = lax.dot_general(wtrows(D + 128 * t), xrows(hf), NT,
                                         preferred_element_type=f32).astype(bf16)
                    for b in range(2):
                        vT_sc[2 + NQ * j + 2 * hf + b, 128 * t:128 * t + 128, :] = vt[:, BQ * b:BQ * b + BQ]

        def tie():
            t = jnp.dot(ms[1 - par][pl.ds(bz_ + F_OFF, ZR), :].astype(bf16), packed(fp_sc, 2),
                        preferred_element_type=f32)
            ms[1 - par][pl.ds(bz_ + F_OFF, ZR), :] = t

        if mode == 'first':
            k_proj(rep=False)
            wait(total(wqv_in, SEM_W))
            start(masks + wo_copy)
            start(k_copy(1) + v_copy(1) + s_copy(1) + x_copy(1) + q_copy(0) + q_copy(1))
            start(k_copy(2) + v_copy(2) + s_copy(2) + x_copy(2))
            init_weights()
            q_proj()
            wait(small + s_wait(0) + k_copy(0) + v_copy(0))
            shk = shk_in[...].astype(f32)
            dvec = d_in[...].astype(f32).reshape(1, D)
            for cc in range(NC):
                par_sc[cc] = jnp.concatenate([shk[:, 128 * cc:128 * cc + 128], dvec[:, 128 * cc:128 * cc + 128],
                                              jnp.zeros((3, 128), f32)], axis=0)
            for s in range(NB):
                g_piece(s)
                u_piece(s)
            k_proj(mm=False)
            zrun(par, zlist(0, ZH[par]))
            v_proj()
            tie()
        elif mode == 'mid':
            for s in range(4):
                g_piece(s)
            outproj(1, j - 1)
            for s in range(NB):
                if s + 4 < NB:
                    g_piece(s + 4)
                u_piece(s)
            if par == 1:
                zrun(0, zlist(ZH[0], 10 ** 6))
                k_proj()
                outproj(2, j - 1)
                for t1 in range(NB):
                    inverse(0, j - 1, t1)
                zrun(1, zlist(0, 10 ** 6))
                q_proj()
                v_proj()
                outproj(3, j - 1)
                for t1 in range(NB):
                    inverse(1, j, t1)
                a_copy(j - 1, 0).start()
                a_copy(j, 1).start()
            else:
                zrun(0, zlist(0, ZH[0]))
                k_proj()
                outproj(2, j - 1)
                q_proj()
                v_proj()
                outproj(3, j - 1)
                tie()
            b_copy(j - 1).start()
        else:
            last = [pltpu.make_async_copy(
                outb_sc.at[(NSTEP - 1) % 2, pl.ds(BQ * b, BQ), :],
                out_hbm.at[0, pl.ds((NSTEP - 1) * RB + BQ * b, BQ), pl.ds(D, D)], sems.at[SEM_X + b])
                for b in range(NQ)]
            for b in range(NQ):
                if b > 0:
                    outproj(b, NSTEP - 1)
                last[b].start()
            a_copy(NSTEP - 2, 0).wait()
            a_copy(NSTEP - 1, 1).wait()
            b_copy(NSTEP - 2).wait()
            wait(last)

    @pl.when(j == 0)
    def _():
        start(wk_copy + x_copy(0))
        wait(total(wk_in, SEM_WK))
        start(w_copy)
        wait(x_wait(0))
        start(small + s_copy(0) + k_copy(0) + v_copy(0))
        pphase('first', 0)

    for js_ in range(1, NSTEP):
        @pl.when(j == js_)
        def _(js_=js_):
            wait(k_copy(js_) + v_copy(js_) + s_wait(js_) + x_wait(js_))
            if js_ % 2 == 1:
                wait(q_copy(js_ - 1) + q_copy(js_))
            if js_ == 2:
                start(k_copy(3) + v_copy(3) + s_copy(3) + x_copy(3) + q_copy(2) + q_copy(3))
                a_copy(0, 0).wait()
                a_copy(1, 1).wait()
            if js_ > 1:
                b_copy(js_ - 2).wait()

    @pl.when(j % 2 == 1)
    def _():
        pphase('mid', 1)

    @pl.when(jnp.logical_and(j % 2 == 0, j > 0))
    def _():
        pphase('mid', 0)

    slot16 = lax.broadcasted_iota(jnp.int32, (16, 128), 1) // 16
    rho56 = lax.broadcasted_iota(jnp.int32, (56, 128), 0) // 8
    slot56 = lax.broadcasted_iota(jnp.int32, (56, 128), 1) // 16
    first56 = slot56 <= rho56
    rho112 = lax.broadcasted_iota(jnp.int32, (112, 128), 0) // 16
    slot112 = lax.broadcasted_iota(jnp.int32, (112, 128), 1) // 16
    first112 = slot112 <= rho112

    zf = lax.shift_right_logical(j, 20).astype(f32)

    rrow_dyn = rrow

    def tphase(first):
        j = 0 if first else jdyn
        rrow = 0 if first else rrow_dyn
        def qk(un):
            b, h = un // H, un % H
            head = first and b < 2
            base = rrow + 64 * b
            qh = qT_sc[b, 16 * h:16 * h + 16, :]
            wq = jnp.concatenate([jnp.where(slot16 == sgm, qh, 0.0) for sgm in range(8)], axis=0).astype(bf16)
            last = rep_sc[h, pl.ds(base + 136, 56), :]
            if not head:
                lhs_u = jnp.concatenate([jnp.where(first56, rep_sc[h, pl.ds(base, 56), :], last),
                                         rep_sc[h, pl.ds(base + 56, 80), :]], axis=0)
                spl = (0, 80, 144, 208, 272)
            elif b == 0:
                lhs_u = jnp.concatenate([last, rep_sc[h, pl.ds(base + 128, 8), :]], axis=0)
                spl = (0, 32, 64, 96, 128)
            else:
                lhs_u = jnp.concatenate([last, rep_sc[h, pl.ds(base + 64, 72), :]], axis=0)
                spl = (0, 64, 128, 192, 256)
            return jnp.concatenate([
                jnp.dot(pltpu.bitcast(lhs_u[spl[i] // 2:spl[i + 1] // 2], bf16), wq, preferred_element_type=f32)
                for i in range(4)], axis=0)

        def softmax(un, st):
            b = un // H
            head = first and b < 2
            nlo = 112 if head else 128
            nmid = 0 if (head and b == 0) else 128
            s_lo = st[0:nlo] + (blo_ref[0, 0:112, :] if head else blo_ref[1])
            s_hi = st[nlo + nmid:nlo + nmid + 16] + bhi_ref[...]
            m8 = _tree(jnp.maximum, _rows8(s_lo) + _rows8(s_hi), 2)
            if nmid:
                s_mid = st[nlo:nlo + nmid]
                m8 = jnp.maximum(m8, _tree(jnp.maximum, _rows8(s_mid), 2))
            m = jnp.max(m8, axis=0, keepdims=True)
            p_lo = jnp.exp2(s_lo - m)
            p_hi = jnp.exp2(s_hi - m)
            mid = [jnp.exp2(s_mid - (m - zf))] if nmid else []
            rows = _rows8(p_lo) + (_rows8(mid[0]) if nmid else []) + _rows8(p_hi)
            l = jnp.sum(_tree(jnp.add, rows, 4), axis=0, keepdims=True)
            if head:
                parts = mid + [p_hi, p_lo]
            else:
                parts = [jnp.where(first112, p_lo[0:112], 0.0), p_lo[112:128]] + mid + [
                    p_hi, jnp.where(first112, 0.0, p_lo[0:112])]
            return jnp.concatenate(parts, axis=0).astype(bf16), l

        def pv(un, frame, l):
            b, h = un // H, un % H
            nt = frame.shape[0] // 128
            vh = jnp.concatenate(
                [packed(vT_sc, (NQ * j + b + i, slice(8 * h, 8 * h + 8), slice(None))) for i in range(3 - nt, 3)],
                axis=1)
            ot = jnp.dot(vh, frame, preferred_element_type=f32)
            oT_sc[b, 16 * h:16 * h + 16, :] = ot * (1.0 / l)

        fr = {}
        pend = list(range(NU))
        for n in range(NU):
            fr[n] = softmax(n, qk(n))
            lag = 2 * LAG if (first and n < H) else LAG
            while pend[0] <= n - lag:
                pv(pend[0], *fr.pop(pend[0]))
                pend.pop(0)
        ostat[0] = j % 2
        outproj(0, j)
        for u in pend:
            pv(u, *fr.pop(u))

    @pl.when(j == 0)
    def _():
        wait(total(wo_in, SEM_WO) + masks)
        tphase(True)

    @pl.when(j > 0)
    def _():
        tphase(False)

    @pl.when(j == NSTEP - 1)
    def _fin():
        pphase('final', (NSTEP - 1) % 2)


@jax.jit
def pallas_concat_heads__ssm_conv_h3__sliding_block__prompt_kernel(
    A_q, A_k, A_v, A_shift_k, A_ssm_k, A_ssm_D, B_x, B_wqkv, B_wo):
    f, blo, bhi = _tables()
    bf16, f32, u32 = jnp.bfloat16, jnp.float32, jnp.uint32
    scratch = [
        pltpu.VMEM((2, S, 128), bf16),
        pltpu.VMEM((3, S, 128), bf16),
        pltpu.VMEM((3, S, 128), bf16),
        pltpu.VMEM((4, D), bf16),
        pltpu.VMEM((3, 128, S), bf16),
        pltpu.VMEM((D,), bf16),
        pltpu.VMEM((3, 4, RB, 128), bf16),
        pltpu.VMEM((2, 4, D, 128), bf16),
        pltpu.VMEM((4, D, 128), bf16),
        pltpu.VMEM((4, D, 128), bf16),
        pltpu.VMEM((4, 128, 128), bf16),
        pltpu.VMEM((2, 128, 128), f32),
        pltpu.VMEM((16, 128), f32),
        pltpu.VMEM((4, 2 * D, 128), bf16),
        pltpu.VMEM((NC, 8, 128), f32),
        pltpu.VMEM((8, 256, 128), bf16),
        pltpu.VMEM((H, (S + 256) // 2, 128), u32),
        pltpu.VMEM((NB + 2, D, 128), bf16),
        pltpu.VMEM((NQ, D, 128), f32),
        pltpu.VMEM((M_ROWS, 128), f32),
        pltpu.VMEM((M_ROWS, 128), f32),
        pltpu.VMEM((NQ, D, BQ), f32),
        pltpu.VMEM((2, S, 128), bf16),
        pltpu.VMEM((2, S, 128), bf16),
        pltpu.VMEM((2, RB, D), bf16),
        pltpu.SemaphoreType.DMA((NSEM,)),
    ]
    return pl.pallas_call(
        _kernel,
        grid=(NSTEP,),
        in_specs=[pl.BlockSpec(memory_space=pl.ANY)] * 12,
        out_specs=pl.BlockSpec(memory_space=pl.ANY),
        out_shape=jax.ShapeDtypeStruct((1, S, 2 * D), bf16),
        scratch_shapes=scratch,
        compiler_params=pltpu.CompilerParams(
            dimension_semantics=("arbitrary",),
            vmem_limit_bytes=110 * 1024 * 1024),
    )(A_q, A_k, A_v, A_shift_k.T, A_ssm_k, A_ssm_D, B_x, B_wqkv, B_wo, f, blo, bhi)
```

```python
import math
import numpy as np
import jax
import jax.numpy as jnp
from jax import lax
import jax.experimental.pallas as pl
import jax.experimental.pallas.tpu as pltpu

S = 2048
D = 512
H = 32
DH = 16
BQ = 128
RB = 512
NQ = RB // BQ
NSTEP = S // RB
NB = S // 128
NC = D // 128
BIG = 1e30
QSCALE = (DH ** -0.5) * math.log2(math.e)
NU = NQ * H
LAG = 4
CS, BS = 72, 232
UG = 32 * BS
Z_OFF = 2 * UG
F_OFF = Z_OFF + 4096
M_ROWS = F_OFF + 16
ZR = 16
(SEM_Q, SEM_K, SEM_V, SEM_S, SEM_X) = (0, 4, 8, 12, 16)
(SEM_W, SEM_WK, SEM_WO, SEM_F, SEM_BLO, SEM_BHI, SEM_SHK, SEM_D, SEM_OB, SEM_OA) = range(20, 30)
NSEM = 31
ZH = (544, 1088)


def _tables():
    n = np.arange(128)[None, :]
    fs = []
    for kap in range(2):
        k = (2 * np.arange(64) + kap)[:, None]
        th = 2.0 * np.pi * (k + 0.5) * n / 256.0
        fs.append(np.concatenate([np.cos(th), -np.sin(th)], axis=0))
    f = np.stack(fs)
    finv = np.transpose(f, (0, 2, 1)) / 128.0
    r = np.arange(16)[:, None]
    a = np.arange(128)[None, :]
    sig, alo = a // 16, a % 16
    lo = np.zeros((2, 128, 128), np.float32)
    for rho in range(8):
        first = sig <= rho
        valid = np.where(sig < rho, True,
                 np.where(sig == rho, r > alo,
                  np.where(sig == rho + 1, r <= alo, True)))
        lo[1, 16 * rho:16 * rho + 16] = np.where(valid, 0.0, -BIG)
        lo[0, 16 * rho:16 * rho + 16] = np.where(valid & ~first, 0.0, -BIG)
    hi = np.where((sig > 0) | (r <= alo), 0.0, -BIG).astype(np.float32)
    return (jnp.asarray(np.concatenate([f, finv]), jnp.bfloat16), jnp.asarray(lo), jnp.asarray(hi))


def _tree(op, xs, ways=4):
    accs = []
    for i, x in enumerate(xs):
        if i < ways:
            accs.append(x)
        else:
            accs[i % ways] = op(accs[i % ways], x)
    while len(accs) > 1:
        accs = [op(accs[i], accs[i + 1]) if i + 1 < len(accs) else accs[i] for i in range(0, len(accs), 2)]
    return accs[0]


def _rows8(x):
    return [x[8 * i:8 * i + 8] for i in range(x.shape[0] // 8)]


def _kernel(q_hbm, k_hbm, v_hbm, shk_hbm, ssmk_hbm, ssmd_hbm, x_hbm, wqkv_hbm, wo_hbm,
            f_hbm, blo_hbm, bhi_hbm, out_hbm,
            q_in, k_in, v_in, shk_in, ssmk_in, d_in, x_in, wqv_in, wk_in, wo_in, fp_sc, blo_ref, bhi_ref,
            wT_sc, par_sc, kst_sc, rep_sc, vT_sc, qT_sc, m0_sc, m1_sc, oT_sc, kv_sc,
            outa_sc, outb_sc, sems):
    j = pl.program_id(0)
    ms = (m0_sc, m1_sc)
    f32, bf16, u32 = jnp.float32, jnp.bfloat16, jnp.uint32
    NT = (((1,), (1,)), ((), ()))
    zero = lambda sh: pl.multiple_of(lax.shift_right_logical(j, sh) * 8, 8)
    bz_, bf_ = zero(13), zero(14)
    mu = lambda kap, r, n: (pl.ds(UG * kap + r, n), slice(None))
    mg = lambda kap, r, n: (pl.ds(UG * kap + 16 * BS + r, n), slice(None))
    mz = lambda r, n: (pl.ds(bz_ + Z_OFF + r, n), slice(None))
    rrow = pl.multiple_of((RB // 2) * j, 128)
    packed = lambda ref, idx: pltpu.bitcast(ref.bitcast(u32)[idx], bf16)

    def tiles_copy(src, dst, sem, n):
        return [pltpu.make_async_copy(src.at[:, pl.ds(128 * t, 128)], dst.at[t], sems.at[sem]) for t in range(n)]

    slot = lambda cc: (0, 1, 2, 1)[cc]
    qslot = lambda cc: cc % 2

    def strip_copy(src, dst, sem0, cc, sl):
        return [pltpu.make_async_copy(src.at[0, :, pl.ds(cc * 128, 128)], dst.at[sl], sems.at[sem0 + cc])]

    q_copy = lambda cc: strip_copy(q_hbm, q_in, SEM_Q, cc, qslot(cc))
    k_copy = lambda cc: strip_copy(k_hbm, k_in, SEM_K, cc, slot(cc))
    v_copy = lambda cc: strip_copy(v_hbm, v_in, SEM_V, cc, slot(cc))
    s_copy = lambda cc: [pltpu.make_async_copy(
        ssmk_hbm.at[pl.ds(cc * 128, 128), :], ssmk_in.at[slot(cc)], sems.at[SEM_S + cc])]
    x_copy = lambda st: tiles_copy(x_hbm.at[0, pl.ds(st * RB, RB), :], x_in.at[slot(st)], SEM_X + st, 4)
    whole = lambda src, dst, sem: [pltpu.make_async_copy(src, dst, sems.at[sem])]
    w_copy = (tiles_copy(wqkv_hbm.at[:, pl.ds(0, D)], wqv_in.at[0], SEM_W, 4)
              + tiles_copy(wqkv_hbm.at[:, pl.ds(2 * D, D)], wqv_in.at[1], SEM_W, 4))
    wk_copy = tiles_copy(wqkv_hbm.at[:, pl.ds(D, D)], wk_in, SEM_WK, 4)
    wo_copy = tiles_copy(wo_hbm, wo_in, SEM_WO, 4)
    small = whole(f_hbm, fp_sc, SEM_F) + whole(shk_hbm, shk_in, SEM_SHK) + whole(ssmd_hbm, d_in, SEM_D)
    masks = whole(blo_hbm, blo_ref, SEM_BLO) + whole(bhi_hbm, bhi_ref, SEM_BHI)

    total = lambda buf, sem: [pltpu.make_async_copy(buf, buf, sems.at[sem])]
    s_wait = s_copy
    x_wait = lambda st: total(x_in.at[slot(st)], SEM_X + st)

    def start(cps):
        for cp in cps:
            cp.start()

    def wait(cps):
        for cp in cps:
            cp.wait()

    def b_copy(step):
        return pltpu.make_async_copy(
            outb_sc.at[step % 2], out_hbm.at[0, pl.ds(step * RB, RB), pl.ds(D, D)], sems.at[SEM_OB])

    def a_copy(cc, p):
        return pltpu.make_async_copy(
            outa_sc.at[p], out_hbm.at[0, :, pl.ds(cc * 128, 128)], sems.at[SEM_OA + p])

    ostat = [None]

    def outproj(b, step):
        o = oT_sc[b].T.astype(bf16)
        for nt in range(4):
            r = jnp.dot(o, packed(wo_in, nt), preferred_element_type=f32)
            osl = (step % 2) if isinstance(step, int) else ostat[0]
            outb_sc[osl, BQ * b:BQ * b + BQ, 128 * nt:128 * nt + 128] = r.astype(bf16)

    def init_weights():
        for w in range(2):
            for t in range(4):
                wt = wqv_in[w, t].astype(f32).T.astype(bf16)
                for kt in range(4):
                    wT_sc[kt, D * w + 128 * t:D * w + 128 * t + 128, :] = wt[:, 128 * kt:128 * kt + 128]

    def zlist(lo, hi):
        out, acc = [], 0
        for a_ in range(NB // 2 - 1, -1, -1):
            for kap in range(2):
                for ch in range(64 // ZR):
                    if lo <= acc < hi:
                        out.append((kap, a_, ch))
                    acc += 4 * a_ + 3
        return out

    jdyn = j

    def pphase(mode, par):
        j = {'first': 0, 'final': NSTEP - 1}.get(mode, 2 if par == 0 else jdyn)
        sl = slot(j) if isinstance(j, int) else 1
        ostat[0] = 0
        rrow = (RB // 2) * j if isinstance(j, int) else pl.multiple_of((RB // 2) * j, 128)
        lane = lax.broadcasted_iota(jnp.int32, (BQ, 128), 1)
        l16 = lane % 16
        kvp = lambda p, s: packed(kv_sc, (p, slice(64 * s, 64 * s + 64), slice(None)))
        ffwd = lambda: pltpu.bitcast(fp_sc.bitcast(u32)[0:2].reshape(128, 128), bf16)
        hprev = [None]

        def kv_piece(s):
            cc = j
            taps = par_sc[cc]
            kf = k_in[sl, 128 * s:128 * s + 128, :].astype(f32)
            if s == 0:
                prev = jnp.zeros((8, 128), f32)
            else:
                prev = k_in[sl, 128 * s - 16:128 * s, :].astype(f32)[8:16]
            ext = jnp.concatenate([prev, kf], axis=0)
            acc = kf * taps[0:1, :]
            for tau in range(1, 4):
                acc = acc + pltpu.roll(ext, tau, 0)[8:136] * taps[tau:tau + 1, :]
            kv_sc[par, 128 * s:128 * s + 128, :] = (
                acc * v_in[sl, 128 * s:128 * s + 128, :].astype(f32)).astype(bf16)

        def g_piece(s):
            cc, m_sc = j, ms[par]
            hh = lax.dot_general(ffwd(), ssmk_in[sl, :, 128 * s:128 * s + 128], NT, preferred_element_type=f32)
            hp = hprev[0]
            for kap in range(2):
                hr, hi = hh[128 * kap:128 * kap + 64], hh[128 * kap + 64:128 * kap + 128]
                if hp is None:
                    gr, gi = hr, hi
                else:
                    pr, pi_ = hp[128 * kap:128 * kap + 64], hp[128 * kap + 64:128 * kap + 128]
                    gr, gi = (hr - pi_, hi + pr) if kap == 0 else (hr + pi_, hi - pr)
                m_sc[mg(kap, BS * s, 64)] = gr
                m_sc[mg(kap, BS * s + CS, 64)] = gi - gr
                m_sc[mg(kap, BS * s + 2 * CS, 64)] = gr + gi
            hprev[0] = hh

        def u_piece(s):
            m_sc = ms[par]
            kv_piece(s)
            uu = jnp.dot(ffwd(), kvp(par, s), preferred_element_type=f32)
            for kap in range(2):
                ur, ui = uu[128 * kap:128 * kap + 64], uu[128 * kap + 64:128 * kap + 128]
                m_sc[mu(kap, BS * s, 64)] = ur
                m_sc[mu(kap, BS * s + CS, 64)] = ui
                m_sc[mu(kap, BS * s + 2 * CS, 64)] = ur + ui

        def zunit(p, kap, a, ch, link=False):
            m_sc = ms[p]
            r0 = ZR * ch
            ldu = lambda s: tuple(m_sc[mu(kap, BS * s + CS * i + r0, ZR)] for i in range(3))
            ldg = lambda s: tuple(m_sc[mg(kap, BS * s + CS * i + r0, ZR)] for i in range(3))
            acc = [None, None]

            def mac(o, u, g):
                p = (g[0] * u[2], u[0] * g[1], u[1] * g[2])
                acc[o] = p if acc[o] is None else tuple(x + y for x, y in zip(acc[o], p))

            uhi = ldu(2 * a + 1)
            for dl in range(2 * a + 2):
                g = ldg(dl)
                mac(1, uhi, g)
                if dl <= 2 * a:
                    ulo = ldu(2 * a - dl)
                    mac(0, ulo, g)
                    uhi = ulo
            for o in range(2):
                k1, k2, k3 = acc[o]
                m_sc[mz(256 * (2 * a + o) + 128 * kap + r0, ZR)] = k1 - k3
                m_sc[mz(256 * (2 * a + o) + 128 * kap + 64 + r0, ZR)] = k1 + k2
            if link:
                ms[1 - p][pl.ds(bf_ + F_OFF, ZR), :] = acc[1][0]

        def zrun(p, units):
            for i, z in enumerate(units):
                zunit(p, *z, link=(i == len(units) - 1))

        def inverse(p, cc, t1):
            rows = slice(128 * t1, 128 * t1 + 128)
            finv = jnp.concatenate([packed(fp_sc, 2), packed(fp_sc, 3)], axis=1)
            yy = jnp.dot(finv, ms[p][mz(256 * t1, 256)].astype(bf16), preferred_element_type=f32)
            dd = par_sc[cc, 4:5, :]
            outa_sc[p, rows, :] = (q_in[p, rows, :].astype(f32) * (yy + kvp(p, t1).astype(f32) * dd)).astype(bf16)

        def xrows(hf):
            return jnp.concatenate(
                [packed(x_in, (sl, kt, slice(128 * hf, 128 * hf + 128), slice(None))) for kt in range(4)], axis=1)

        def wtrows(r0):
            return jnp.concatenate(
                [packed(wT_sc, (kt, slice(r0 // 2, r0 // 2 + 64), slice(None))) for kt in range(4)], axis=1)

        def k_mm(g, hf):
            kf = jnp.dot(xrows(hf), packed(wk_in, g), preferred_element_type=f32)
            kst_sc[2 * g + hf] = kf.astype(bf16)

        def k_rep(g, hf):
            kg = kst_sc.bitcast(u32)[2 * g + hf]
            dst = pl.ds(rrow + 128 + 128 * hf, 128)
            for hl in range(8):
                rep_sc[8 * g + hl, dst, :] = jnp.take_along_axis(kg, l16 + 16 * hl, axis=1)

        def k_proj(mm=True, rep=True):
            for hf in range(2):
                for g in range(4):
                    if mm:
                        k_mm(g, hf)
                    if rep:
                        k_rep(g, hf)

        def q_proj():
            for hf in range(2):
                for t in range(4):
                    qt = lax.dot_general(wtrows(128 * t), xrows(hf), NT, preferred_element_type=f32) * QSCALE
                    for b in range(2):
                        qT_sc[2 * hf + b, 128 * t:128 * t + 128, :] = qt[:, BQ * b:BQ * b + BQ]

        def v_proj():
            for hf in range(2):
                for t in range(4):
                    vt = lax.dot_general(wtrows(D + 128 * t), xrows(hf), NT,
                                         preferred_element_type=f32).astype(bf16)
                    for b in range(2):
                        vT_sc[2 + NQ * j + 2 * hf + b, 128 * t:128 * t + 128, :] = vt[:, BQ * b:BQ * b + BQ]

        def tie():
            t = jnp.dot(ms[1 - par][pl.ds(bz_ + F_OFF, ZR), :].astype(bf16), packed(fp_sc, 2),
                        preferred_element_type=f32)
            ms[1 - par][pl.ds(bz_ + F_OFF, ZR), :] = t

        if mode == 'first':
            k_proj(rep=False)
            wait(total(wqv_in, SEM_W))
            start(masks + wo_copy)
            start(k_copy(1) + v_copy(1) + s_copy(1) + x_copy(1) + q_copy(0) + q_copy(1))
            start(k_copy(2) + v_copy(2) + s_copy(2) + x_copy(2))
            init_weights()
            q_proj()
            wait(small + s_wait(0) + k_copy(0) + v_copy(0))
            shk = shk_in[...].astype(f32)
            dvec = d_in[...].astype(f32).reshape(1, D)
            for cc in range(NC):
                par_sc[cc] = jnp.concatenate([shk[:, 128 * cc:128 * cc + 128], dvec[:, 128 * cc:128 * cc + 128],
                                              jnp.zeros((3, 128), f32)], axis=0)
            for s in range(NB):
                g_piece(s)
                u_piece(s)
            k_proj(mm=False)
            zrun(par, zlist(0, ZH[par]))
            v_proj()
            tie()
        elif mode == 'mid':
            for s in range(4):
                g_piece(s)
            outproj(1, j - 1)
            for s in range(NB):
                if s + 4 < NB:
                    g_piece(s + 4)
                u_piece(s)
            if par == 1:
                zrun(0, zlist(ZH[0], 10 ** 6))
                k_proj()
                outproj(2, j - 1)
                for t1 in range(NB):
                    inverse(0, j - 1, t1)
                zrun(1, zlist(0, 10 ** 6))
                q_proj()
                v_proj()
                outproj(3, j - 1)
                for t1 in range(NB):
                    inverse(1, j, t1)
                a_copy(j - 1, 0).start()
                a_copy(j, 1).start()
            else:
                zrun(0, zlist(0, ZH[0]))
                k_proj()
                outproj(2, j - 1)
                q_proj()
                v_proj()
                outproj(3, j - 1)
                tie()
            b_copy(j - 1).start()
        else:
            last = [pltpu.make_async_copy(
                outb_sc.at[(NSTEP - 1) % 2, pl.ds(BQ * b, BQ), :],
                out_hbm.at[0, pl.ds((NSTEP - 1) * RB + BQ * b, BQ), pl.ds(D, D)], sems.at[SEM_X + b])
                for b in range(NQ)]
            for b in range(NQ):
                if b > 0:
                    outproj(b, NSTEP - 1)
                last[b].start()
            a_copy(NSTEP - 2, 0).wait()
            a_copy(NSTEP - 1, 1).wait()
            b_copy(NSTEP - 2).wait()
            wait(last)

    @pl.when(j == 0)
    def _():
        start(wk_copy + x_copy(0))
        vT_sc[...] = jnp.zeros(vT_sc.shape, bf16)
        kv_sc[...] = jnp.zeros(kv_sc.shape, bf16)
        wait(total(wk_in, SEM_WK))
        start(w_copy)
        kst_sc[...] = jnp.zeros(kst_sc.shape, bf16)
        wT_sc[...] = jnp.zeros(wT_sc.shape, bf16)
        x_in[1:3] = jnp.zeros((2,) + x_in.shape[1:], bf16)
        wait(x_wait(0))
        start(small + s_copy(0) + k_copy(0) + v_copy(0))
        pphase('first', 0)

    for js_ in range(1, NSTEP):
        @pl.when(j == js_)
        def _(js_=js_):
            wait(k_copy(js_) + v_copy(js_) + s_wait(js_) + x_wait(js_))
            if js_ % 2 == 1:
                wait(q_copy(js_ - 1) + q_copy(js_))
            if js_ == 2:
                start(k_copy(3) + v_copy(3) + s_copy(3) + x_copy(3) + q_copy(2) + q_copy(3))
                a_copy(0, 0).wait()
                a_copy(1, 1).wait()
            if js_ > 1:
                b_copy(js_ - 2).wait()

    @pl.when(j % 2 == 1)
    def _():
        pphase('mid', 1)

    @pl.when(jnp.logical_and(j % 2 == 0, j > 0))
    def _():
        pphase('mid', 0)

    slot16 = lax.broadcasted_iota(jnp.int32, (16, 128), 1) // 16
    rho56 = lax.broadcasted_iota(jnp.int32, (56, 128), 0) // 8
    slot56 = lax.broadcasted_iota(jnp.int32, (56, 128), 1) // 16
    first56 = slot56 <= rho56
    rho112 = lax.broadcasted_iota(jnp.int32, (112, 128), 0) // 16
    slot112 = lax.broadcasted_iota(jnp.int32, (112, 128), 1) // 16
    first112 = slot112 <= rho112

    zf = lax.shift_right_logical(j, 20).astype(f32)

    rrow_dyn = rrow

    def tphase(first):
        j = 0 if first else jdyn
        rrow = 0 if first else rrow_dyn
        def qk(un):
            b, h = un // H, un % H
            head = first and b < 2
            base = rrow + 64 * b
            qh = qT_sc[b, 16 * h:16 * h + 16, :]
            wq = jnp.concatenate([jnp.where(slot16 == sgm, qh, 0.0) for sgm in range(8)], axis=0).astype(bf16)
            last = rep_sc[h, pl.ds(base + 136, 56), :]
            if not head:
                lhs_u = jnp.concatenate([jnp.where(first56, rep_sc[h, pl.ds(base, 56), :], last),
                                         rep_sc[h, pl.ds(base + 56, 80), :]], axis=0)
                spl = (0, 80, 144, 208, 272)
            elif b == 0:
                lhs_u = jnp.concatenate([last, rep_sc[h, pl.ds(base + 128, 8), :]], axis=0)
                spl = (0, 32, 64, 96, 128)
            else:
                lhs_u = jnp.concatenate([last, rep_sc[h, pl.ds(base + 64, 72), :]], axis=0)
                spl = (0, 64, 128, 192, 256)
            return jnp.concatenate([
                jnp.dot(pltpu.bitcast(lhs_u[spl[i] // 2:spl[i + 1] // 2], bf16), wq, preferred_element_type=f32)
                for i in range(4)], axis=0)

        def softmax(un, st):
            b = un // H
            head = first and b < 2
            nlo = 112 if head else 128
            nmid = 0 if (head and b == 0) else 128
            s_lo = st[0:nlo] + (blo_ref[0, 0:112, :] if head else blo_ref[1])
            s_hi = st[nlo + nmid:nlo + nmid + 16] + bhi_ref[...]
            m8 = _tree(jnp.maximum, _rows8(s_lo) + _rows8(s_hi), 2)
            if nmid:
                s_mid = st[nlo:nlo + nmid]
                m8 = jnp.maximum(m8, _tree(jnp.maximum, _rows8(s_mid), 2))
            m = jnp.max(m8, axis=0, keepdims=True)
            p_lo = jnp.exp2(s_lo - m)
            p_hi = jnp.exp2(s_hi - m)
            mid = [jnp.exp2(s_mid - (m - zf))] if nmid else []
            rows = _rows8(p_lo) + (_rows8(mid[0]) if nmid else []) + _rows8(p_hi)
            l = jnp.sum(_tree(jnp.add, rows, 4), axis=0, keepdims=True)
            if head:
                parts = mid + [p_hi, p_lo]
            else:
                parts = [jnp.where(first112, p_lo[0:112], 0.0), p_lo[112:128]] + mid + [
                    p_hi, jnp.where(first112, 0.0, p_lo[0:112])]
            return jnp.concatenate(parts, axis=0).astype(bf16), l

        def pv(un, frame, l):
            b, h = un // H, un % H
            nt = frame.shape[0] // 128
            vh = jnp.concatenate(
                [packed(vT_sc, (NQ * j + b + i, slice(8 * h, 8 * h + 8), slice(None))) for i in range(3 - nt, 3)],
                axis=1)
            ot = jnp.dot(vh, frame, preferred_element_type=f32)
            oT_sc[b, 16 * h:16 * h + 16, :] = ot * (1.0 / l)

        fr = {}
        pend = list(range(NU))
        for n in range(NU):
            fr[n] = softmax(n, qk(n))
            lag = 2 * LAG if (first and n < H) else LAG
            while pend[0] <= n - lag:
                pv(pend[0], *fr.pop(pend[0]))
                pend.pop(0)
        ostat[0] = j % 2
        outproj(0, j)
        for u in pend:
            pv(u, *fr.pop(u))

    @pl.when(j == 0)
    def _():
        wait(total(wo_in, SEM_WO) + masks)
        tphase(True)

    @pl.when(j > 0)
    def _():
        tphase(False)

    @pl.when(j == NSTEP - 1)
    def _fin():
        pphase('final', (NSTEP - 1) % 2)


@jax.jit
def pallas_concat_heads__ssm_conv_h3__sliding_block__prompt_kernel(
    A_q, A_k, A_v, A_shift_k, A_ssm_k, A_ssm_D, B_x, B_wqkv, B_wo):
    f, blo, bhi = _tables()
    bf16, f32, u32 = jnp.bfloat16, jnp.float32, jnp.uint32
    scratch = [
        pltpu.VMEM((2, S, 128), bf16),
        pltpu.VMEM((3, S, 128), bf16),
        pltpu.VMEM((3, S, 128), bf16),
        pltpu.VMEM((4, D), bf16),
        pltpu.VMEM((3, 128, S), bf16),
        pltpu.VMEM((D,), bf16),
        pltpu.VMEM((3, 4, RB, 128), bf16),
        pltpu.VMEM((2, 4, D, 128), bf16),
        pltpu.VMEM((4, D, 128), bf16),
        pltpu.VMEM((4, D, 128), bf16),
        pltpu.VMEM((4, 128, 128), bf16),
        pltpu.VMEM((2, 128, 128), f32),
        pltpu.VMEM((16, 128), f32),
        pltpu.VMEM((4, 2 * D, 128), bf16),
        pltpu.VMEM((NC, 8, 128), f32),
        pltpu.VMEM((8, 256, 128), bf16),
        pltpu.VMEM((H, (S + 256) // 2, 128), u32),
        pltpu.VMEM((NB + 2, D, 128), bf16),
        pltpu.VMEM((NQ, D, 128), f32),
        pltpu.VMEM((M_ROWS, 128), f32),
        pltpu.VMEM((M_ROWS, 128), f32),
        pltpu.VMEM((NQ, D, BQ), f32),
        pltpu.VMEM((2, S, 128), bf16),
        pltpu.VMEM((2, S, 128), bf16),
        pltpu.VMEM((2, RB, D), bf16),
        pltpu.SemaphoreType.DMA((NSEM,)),
    ]
    return pl.pallas_call(
        _kernel,
        grid=(NSTEP,),
        in_specs=[pl.BlockSpec(memory_space=pl.ANY)] * 12,
        out_specs=pl.BlockSpec(memory_space=pl.ANY),
        out_shape=jax.ShapeDtypeStruct((1, S, 2 * D), bf16),
        scratch_shapes=scratch,
        compiler_params=pltpu.CompilerParams(
            dimension_semantics=("arbitrary",),
            vmem_limit_bytes=110 * 1024 * 1024),
    )(A_q, A_k, A_v, A_shift_k.T, A_ssm_k, A_ssm_D, B_x, B_wqkv, B_wo, f, blo, bhi)
```
